```python
import os as _os
_os.environ.setdefault("JAX_PLATFORMS", "cpu")
import jax
import jax.numpy as jnp

def _softmax(x, axis=-1):
    return jax.nn.softmax(x, axis=axis)
def _gelu(x):
    return jax.nn.gelu(x, approximate=True)
def _silu(x):
    return jax.nn.silu(x)
def _sigmoid(x):
    return jax.nn.sigmoid(x)
def _layernorm(x, axis=-1, eps=1e-5):
    m = jnp.mean(x, axis=axis, keepdims=True)
    v = jnp.var(x, axis=axis, keepdims=True)
    return (x - m) / jnp.sqrt(v + eps)
def _scatter_add(tgt, idx, src, axis=0):
    return tgt.at[idx].add(src)
def _segment_sum(src, seg, n):
    return jax.ops.segment_sum(src, seg, n)
class _Rng:
    def __init__(self, key):
        self._k = key
    def _next(self):
        self._k, sub = jax.random.split(self._k)
        return sub
    def normal(self, shape):
        return jax.random.normal(self._next(), shape, dtype=jnp.bfloat16)
    def randint(self, lo, hi, shape):
        return jax.random.randint(self._next(), shape, lo, hi, dtype=jnp.int32)
    def uniform(self, shape, lo=0.0, hi=1.0):
        return jax.random.uniform(self._next(), shape, jnp.bfloat16, lo, hi)
    def permutation(self, n):
        return jax.random.permutation(self._next(), n)


kernel_name = 'standalone__mha_block_cached__near_ridge'

def setup_inputs():
    _rng = _Rng(jax.random.key(int.from_bytes(__import__("os").urandom(4), "little")))
    _w = (lambda a: (lambda t: t.astype(jnp.bfloat16) if jnp.issubdtype(t.dtype, jnp.floating) else t)(jnp.asarray(a)))
    B, Sq, D = 8, 96, 576
    H, Sk, Dh = 32, 96, 128
    return {
        "x": _w((lambda *s: _rng.normal(s) * 0.8)(B, Sq, D)),
        "k_cache": _w((lambda *s: _rng.normal(s) * 0.8)(B, H, Sk, Dh)),
        "v_cache": _w((lambda *s: _rng.normal(s) * 0.05)(B, H, Sk, Dh)),
        "wq": _w((lambda *s: _rng.normal(s) * 0.8)(D, H * Dh) * (D ** -0.5)),
        "wo": _w((lambda *s: _rng.normal(s) * 0.05)(H * Dh, D) * ((H * Dh) ** -0.5)),
    }

def reference(x, k_cache, v_cache, wq, wo):
    B, Sq, D = x.shape
    H, Dh = 32, 128
    q = (lambda x, *d: x.transpose(*d))((x @ wq).reshape(B, Sq, H, Dh), 0, 2, 1, 3)
    scores = jnp.einsum("bhqd,bhkd->bhqk", q, k_cache) * (Dh ** -0.5)
    p = _softmax(scores, axis=-1)
    o = jnp.einsum("bhqk,bhkd->bhqd", p, v_cache)
    return (lambda x, *d: x.transpose(*d))(o, 0, 2, 1, 3).reshape(B, Sq, H * Dh) @ wo
```

```python
import functools

import jax
import jax.numpy as jnp
from jax import lax
import jax.experimental.pallas as pl
import jax.experimental.pallas.tpu as pltpu

B, SQ, D, H, SK, DH = 8, 96, 576, 32, 96, 128
M = B * SQ
G = 4
NG = H // G
W = G * DH
OC = 128
NC = M // OC
X0 = 256
HS = 8
SPLIT = 2
SCALE_LOG2E = (DH ** -0.5) * 1.4426950408889634
NT = (((1,), (1,)), ((), ()))
f32, bf16 = jnp.float32, jnp.bfloat16


def _kernel(x_hbm, k_hbm, v_hbm, wq_hbm, wot_hbm, out_hbm,
            x_v, k_v, v_v, wq_v, wot_v, q_v, o_v, out_v, sems):
    def cp(src, dst, i):
        return pltpu.make_async_copy(src, dst, sems.at[i])

    def cx(r0, n, i):
        return [cp(x_hbm.at[pl.ds(r0, n)], x_v.at[pl.ds(r0, n)], i)]

    def cwq(g0, g1, i):
        return [cp(wq_hbm.at[:, pl.ds(g * W, W)], wq_v.at[g], i) for g in range(g0, g1)]

    def ckv(b0, n, i):
        return [cp(k_hbm.at[pl.ds(b0, n)], k_v.at[pl.ds(b0, n)], i),
                cp(v_hbm.at[pl.ds(b0, n)], v_v.at[pl.ds(b0, n)], i)]

    def cout(r0, n, i):
        return cp(out_v.at[pl.ds(r0, n)], out_hbm.at[pl.ds(r0, n)], i)

    sets = [
        cwq(0, 1, 0) + cx(0, X0, 0),
        cx(X0, M - X0, 1),
        cwq(1, 3, 2),
        cwq(3, 5, 3),
        cwq(5, NG, 4) + ckv(0, 2, 4),
        [cp(wot_hbm, wot_v, 5)] + ckv(2, 2, 5),
        ckv(4, 4, 6),
    ]

    def once(fn):
        def body(i, carry):
            fn()
            return carry
        lax.fori_loop(0, 1 + pl.program_id(0), body, 0)

    def start(i):
        for c in sets[i]:
            c.start()

    def wait(i):
        for c in sets[i]:
            c.wait()

    def qproj(g, r0, n):
        r = pl.ds(r0, n)
        q_v[g, r, :] = jnp.dot(x_v[r, :], wq_v[g], preferred_element_type=f32).astype(bf16)

    def scores(b, h):
        hh = h % G
        q = q_v[h // G, b * SQ:(b + 1) * SQ, hh * DH:(hh + 1) * DH]
        return lax.dot_general(q, k_v[b, h], NT, preferred_element_type=f32)

    def softmax_parts(s):
        m = jnp.max(s, axis=-1, keepdims=True)
        p = jnp.exp2((s - m) * SCALE_LOG2E)
        l = jnp.sum(p, axis=-1, keepdims=True)
        r = pl.reciprocal(l, approx=True)
        r = r * (2.0 - l * r)
        return p.astype(bf16), r

    def pv(b, h, pr):
        p, r = pr
        hh = h % G
        o = jnp.dot(p, v_v[b, h], preferred_element_type=f32) * r
        o_v[h // G, b * SQ:(b + 1) * SQ, hh * DH:(hh + 1) * DH] = o.astype(bf16)

    def attend(bs, fillers):
        items = [(b, h) for b in bs for h in range(H)]
        stages = [items[i:i + HS] for i in range(0, len(items), HS)]
        n = len(stages)

        def stage(i):
            ss = [scores(b, h) for b, h in stages[i]]
            return [softmax_parts(s) for s in ss]

        cur = stage(0)
        for i in range(n):
            nxt = stage(i + 1) if i + 1 < n else None
            for fill in fillers[i * len(fillers) // n:(i + 1) * len(fillers) // n]:
                fill()
            for (b, h), pr in zip(stages[i], cur):
                pv(b, h, pr)
            cur = nxt

    def ochunk(c):
        st = {}
        rows = slice(c * OC, (c + 1) * OC)

        def part(g):
            t = lax.dot_general(wot_v[:, g * W:(g + 1) * W], o_v[g, rows, :], NT,
                                preferred_element_type=f32)
            st["acc"] = t if g == 0 else st["acc"] + t
            if g == NG - 1:
                out_v[rows, :] = st.pop("acc").astype(bf16).T

        return [functools.partial(part, g) for g in range(NG)]

    def run(fns):
        for fn in fns:
            fn()

    start(0)
    for i in range(1, len(sets)):
        once(functools.partial(start, i))

    wait(0)
    qproj(0, 0, X0)
    wait(1)
    qproj(0, X0, M - X0)
    wait(2)
    qproj(1, 0, M)
    qproj(2, 0, M)
    wait(3)
    qproj(3, 0, M)
    qproj(4, 0, M)
    wait(4)
    qproj(5, 0, M)
    qproj(6, 0, 2 * SQ)
    qproj(7, 0, 2 * SQ)
    attend([0, 1], [functools.partial(qproj, g, r, 2 * SQ)
                    for r in range(2 * SQ, M, 2 * SQ) for g in (6, 7)])
    wait(5)
    attend([2, 3], ochunk(0))
    c1 = ochunk(1)
    run(c1[:NG - SPLIT])
    wait(6)
    attend([4, 5], c1[NG - SPLIT:] + ochunk(2))
    attend([6, 7], ochunk(3))
    run(ochunk(4))
    c5 = ochunk(5)
    run(c5[:SPLIT])
    head, tail = cout(0, M - OC, 0), cout(M - OC, OC, 1)
    once(head.start)
    run(c5[SPLIT:])
    tail.start()
    head.wait()
    tail.wait()


@jax.jit
def pallas_standalone__mha_block_cached__near_ridge_kernel(
    x: jax.Array,
    k_cache: jax.Array,
    v_cache: jax.Array,
    wq: jax.Array,
    wo: jax.Array,
):
    hbm = pl.BlockSpec(memory_space=pltpu.HBM)
    out = pl.pallas_call(
        _kernel,
        grid=(1,),
        out_shape=jax.ShapeDtypeStruct((M, D), bf16),
        in_specs=[hbm] * 5,
        out_specs=hbm,
        scratch_shapes=[
            pltpu.VMEM((M, D), bf16),
            pltpu.VMEM((B, H, SK, DH), bf16),
            pltpu.VMEM((B, H, SK, DH), bf16),
            pltpu.VMEM((NG, D, W), bf16),
            pltpu.VMEM((D, H * DH), bf16),
            pltpu.VMEM((NG, M, W), bf16),
            pltpu.VMEM((NG, M, W), bf16),
            pltpu.VMEM((M, D), bf16),
            pltpu.SemaphoreType.DMA((7,)),
        ],
        compiler_params=pltpu.CompilerParams(vmem_limit_bytes=100 * 1024 * 1024),
    )(x.reshape(M, D), k_cache, v_cache, wq, wo.T)
    return out.reshape(B, SQ, D)
```

```python
import functools

import jax
import jax.numpy as jnp
from jax import lax
import jax.experimental.pallas as pl
import jax.experimental.pallas.tpu as pltpu

B, SQ, D, H, SK, DH = 8, 96, 576, 32, 96, 128
M = B * SQ
G = 4
NG = H // G
W = G * DH
OC = 128
NC = M // OC
NK = 2
HS = 8
SPLIT = 2
SCALE_LOG2E = (DH ** -0.5) * 1.4426950408889634
NT = (((1,), (1,)), ((), ()))
f32, bf16 = jnp.float32, jnp.bfloat16


def _kernel(x_hbm, k_hbm, v_hbm, wq_hbm, wot_hbm, out_hbm,
            x_v, k_v, v_v, wq_v, wot_v, q_v, o_v, out_v, a_v, sems):
    def cp(src, dst, i):
        return pltpu.make_async_copy(src, dst, sems.at[i])

    def cxk(k0, k1, i):
        ks = pl.ds(k0, k1 - k0)
        return [cp(x_hbm.at[:, ks], x_v.at[:, ks], i)] + [
            cp(wq_hbm.at[ks, pl.ds(g * W, W)], wq_v.at[g, ks], i) for g in range(NK)]

    def cwq(g0, g1, i):
        return [cp(wq_hbm.at[:, pl.ds(g * W, W)], wq_v.at[g], i) for g in range(g0, g1)]

    def ckv(b0, n, i):
        return [cp(k_hbm.at[pl.ds(b0, n)], k_v.at[pl.ds(b0, n)], i),
                cp(v_hbm.at[pl.ds(b0, n)], v_v.at[pl.ds(b0, n)], i)]

    def cout(r0, n, i):
        return cp(out_v.at[pl.ds(r0, n)], out_hbm.at[pl.ds(r0, n)], i)

    sets = [
        cxk(0, 128, 0),
        cxk(128, 384, 1),
        cxk(384, D, 2) + cwq(2, 3, 2),
        cwq(3, 5, 3),
        cwq(5, NG, 4) + ckv(0, 2, 4),
        [cp(wot_hbm, wot_v, 5)] + ckv(2, 2, 5),
        ckv(4, 4, 6),
    ]

    def once(fn):
        def body(i, carry):
            fn()
            return carry
        lax.fori_loop(0, 1 + pl.program_id(0), body, 0)

    def start(i):
        for c in sets[i]:
            c.start()

    def wait(i):
        for c in sets[i]:
            c.wait()

    def st(ref, g, r0, n, cols, val):
        ref[g, r0 // 2:(r0 + n) // 2, cols] = pltpu.bitcast(val.astype(bf16), jnp.uint32)

    def ld(ref, g, r0, n, cols):
        return pltpu.bitcast(ref[g, r0 // 2:(r0 + n) // 2, cols], bf16)

    def qproj(g, r0, n):
        t = jnp.dot(x_v[r0:r0 + n, :], wq_v[g], preferred_element_type=f32)
        st(q_v, g, r0, n, slice(None), t)

    def qproj_partial(k0, k1):
        for g in range(NK):
            t = jnp.dot(x_v[:, k0:k1], wq_v[g, k0:k1, :], preferred_element_type=f32)
            if k0 > 0:
                t = t + a_v[g]
            if k1 < D:
                a_v[g] = t
            else:
                st(q_v, g, 0, M, slice(None), t)

    def scores(b, h):
        hh = h % G
        q = ld(q_v, h // G, b * SQ, SQ, slice(hh * DH, (hh + 1) * DH))
        return lax.dot_general(q, k_v[b, h], NT, preferred_element_type=f32)

    def softmax_parts(s):
        m = jnp.max(s, axis=-1, keepdims=True)
        p = jnp.exp2((s - m) * SCALE_LOG2E)
        l = jnp.sum(p, axis=-1, keepdims=True)
        r = pl.reciprocal(l, approx=True)
        r = r * (2.0 - l * r)
        return p.astype(bf16), r

    def pv(b, h, pr):
        p, r = pr
        hh = h % G
        o = jnp.dot(p, v_v[b, h], preferred_element_type=f32) * r
        st(o_v, h // G, b * SQ, SQ, slice(hh * DH, (hh + 1) * DH), o)

    def attend(bs, fillers):
        items = [(b, h) for b in bs for h in range(H)]
        stages = [items[i:i + HS] for i in range(0, len(items), HS)]
        n = len(stages)

        def stage(i):
            ss = [scores(b, h) for b, h in stages[i]]
            return [softmax_parts(s) for s in ss]

        cur = stage(0)
        for i in range(n):
            nxt = stage(i + 1) if i + 1 < n else None
            for fill in fillers[i * len(fillers) // n:(i + 1) * len(fillers) // n]:
                fill()
            for (b, h), pr in zip(stages[i], cur):
                pv(b, h, pr)
            cur = nxt

    def ochunk(c):
        acc = {}
        rows = slice(c * OC, (c + 1) * OC)

        def part(g):
            t = lax.dot_general(wot_v[:, g * W:(g + 1) * W],
                                ld(o_v, g, c * OC, OC, slice(None)), NT,
                                preferred_element_type=f32)
            acc["t"] = t if g == 0 else acc["t"] + t
            if g == NG - 1:
                out_v[rows, :] = acc.pop("t").astype(bf16).T

        return [functools.partial(part, g) for g in range(NG)]

    def run(fns):
        for fn in fns:
            fn()

    start(0)
    for i in range(1, len(sets)):
        once(functools.partial(start, i))

    wait(0)
    qproj_partial(0, 128)
    wait(1)
    qproj_partial(128, 384)
    wait(2)
    qproj_partial(384, D)
    qproj(2, 0, M)
    wait(3)
    qproj(3, 0, M)
    qproj(4, 0, M)
    wait(4)
    qproj(5, 0, M)
    qproj(6, 0, 2 * SQ)
    qproj(7, 0, 2 * SQ)
    attend([0, 1], [functools.partial(qproj, g, r, 2 * SQ)
                    for r in range(2 * SQ, M, 2 * SQ) for g in (6, 7)])
    wait(5)
    attend([2, 3], ochunk(0))
    c1 = ochunk(1)
    run(c1[:NG - SPLIT])
    wait(6)
    attend([4, 5], c1[NG - SPLIT:] + ochunk(2))
    attend([6, 7], ochunk(3))
    run(ochunk(4))
    c5 = ochunk(5)
    run(c5[:SPLIT])
    head, tail = cout(0, M - OC, 0), cout(M - OC, OC, 1)
    once(head.start)
    run(c5[SPLIT:])
    tail.start()
    head.wait()
    tail.wait()


@jax.jit
def pallas_standalone__mha_block_cached__near_ridge_kernel(
    x: jax.Array,
    k_cache: jax.Array,
    v_cache: jax.Array,
    wq: jax.Array,
    wo: jax.Array,
):
    hbm = pl.BlockSpec(memory_space=pltpu.HBM)
    out = pl.pallas_call(
        _kernel,
        grid=(1,),
        out_shape=jax.ShapeDtypeStruct((M, D), bf16),
        in_specs=[hbm] * 5,
        out_specs=hbm,
        scratch_shapes=[
            pltpu.VMEM((M, D), bf16),
            pltpu.VMEM((B, H, SK, DH), bf16),
            pltpu.VMEM((B, H, SK, DH), bf16),
            pltpu.VMEM((NG, D, W), bf16),
            pltpu.VMEM((D, H * DH), bf16),
            pltpu.VMEM((NG, M // 2, W), jnp.uint32),
            pltpu.VMEM((NG, M // 2, W), jnp.uint32),
            pltpu.VMEM((M, D), bf16),
            pltpu.VMEM((NK, M, W), f32),
            pltpu.SemaphoreType.DMA((7,)),
        ],
        compiler_params=pltpu.CompilerParams(vmem_limit_bytes=100 * 1024 * 1024),
    )(x.reshape(M, D), k_cache, v_cache, wq, wo.T)
    return out.reshape(B, SQ, D)
```
